```python
import jax
import jax.numpy as jnp

def _softmax(x, axis=-1):
    return jax.nn.softmax(x, axis=axis)
def _gelu(x):
    return jax.nn.gelu(x, approximate=True)
def _silu(x):
    return jax.nn.silu(x)
def _sigmoid(x):
    return jax.nn.sigmoid(x)
def _layernorm(x, axis=-1, eps=1e-5):
    m = jnp.mean(x, axis=axis, keepdims=True)
    v = jnp.var(x, axis=axis, keepdims=True)
    return (x - m) / jnp.sqrt(v + eps)
def _scatter_add(tgt, idx, src, axis=0):
    return tgt.at[idx].add(src)
def _segment_sum(src, seg, n):
    return jax.ops.segment_sum(src, seg, n)
class _Rng:
    def __init__(self, key):
        self._k = key
    def _next(self):
        self._k, sub = jax.random.split(self._k)
        return sub
    def normal(self, shape):
        return jax.random.normal(self._next(), shape, dtype=jnp.bfloat16)
    def randint(self, lo, hi, shape):
        return jax.random.randint(self._next(), shape, lo, hi, dtype=jnp.int32)
    def uniform(self, shape, lo=0.0, hi=1.0):
        return jax.random.uniform(self._next(), shape, jnp.bfloat16, lo, hi)
    def permutation(self, n):
        return jax.random.permutation(self._next(), n)


kernel_name = 'sequential_preLN__spectral_gfnet__swiglu_ffn__prompt'

def _fwd_setup_inputs():
    _rng = _Rng(jax.random.key(int.from_bytes(__import__("os").urandom(4), "little")))
    _w = (lambda a: (lambda t: t.astype(jnp.bfloat16) if jnp.issubdtype(t.dtype, jnp.floating) else t)(jnp.asarray(a)))
    def _A_setup():
        B, S, D = 1, 2048, 576
        Df = D // 2 + 1
        return {
            "x": _w((lambda *s: _rng.normal(s) * 0.05)(B, S, D)),
            "w_r": _w((lambda *s: _rng.normal(s) * 0.05)(S, Df) * 0.02),
            "w_i": _w((lambda *s: _rng.normal(s) * 0.05)(S, Df) * 0.02),
        }
    _A_in = _A_setup()

    def _B_setup():
        B, S, D, F = 1, 2048, 576, 4608
        return {
            "x": _w((lambda *s: _rng.normal(s) * 0.05)(B, S, D)),
            "w_gate": _w((lambda *s: _rng.normal(s) * 0.05)(D, F)),
            "w_up": _w((lambda *s: _rng.normal(s) * 0.05)(D, F)),
            "w_down": _w((lambda *s: _rng.normal(s) * 0.05)(F, D)),
        }
    _B_in = _B_setup()

    return {
        "A_x": _A_in["x"],
        "A_w_r": _A_in["w_r"],
        "A_w_i": _A_in["w_i"],
        "B_x": _B_in["x"],
        "B_w_gate": _B_in["w_gate"],
        "B_w_up": _B_in["w_up"],
        "B_w_down": _B_in["w_down"],
    }

def _fwd_reference(A_x, A_w_r, A_w_i, B_x, B_w_gate, B_w_up, B_w_down):
    def _A_ref(x, w_r, w_i):
        B, S, D = x.shape
        X = (lambda x, axes=(-2,-1): jnp.fft.rfft2(x.astype(jnp.float32), axes=axes))(x, axes=(-2, -1))
        W = w_r + 1j * w_i
        X = X * W
        y = (lambda x, s, axes=(-2,-1): jnp.fft.irfft2(x, s=s, axes=axes).astype(jnp.bfloat16))(X, (S, D), axes=(-2, -1))
        return y

    def _B_ref(x, w_gate, w_up, w_down):
        g = _silu(x @ w_gate)
        u = x @ w_up
        return (g * u) @ w_down

    x = A_x
    h = x + _A_ref(_layernorm(x, axis=-1), A_w_r, A_w_i)
    h2 = h + _B_ref(_layernorm(h, axis=-1), B_w_gate, B_w_up, B_w_down)
    return h2


def setup_inputs():
    _inp = _fwd_setup_inputs()
    _gk = jax.random.fold_in(jax.random.key(int.from_bytes(__import__("os").urandom(4), "little")), 2**31 - 1)
    _shapes = [[1, 2048, 576]]
    _dtypes = ['bfloat16']
    _gks = jax.random.split(_gk, len(_shapes))
    _gs = [jax.random.normal(k, s, dtype=jnp.dtype(d)) * 0.05 for k, s, d in zip(_gks, _shapes, _dtypes)]
    _inp["grad_out"] = _gs[0]
    return _inp

def reference(A_x, A_w_r, A_w_i, B_w_gate, B_w_up, B_w_down, B_x, grad_out):
    _const = dict(B_x=B_x)
    def _f(*_d):
        return _fwd_reference(**{'A_x': _d[0], 'A_w_r': _d[1], 'A_w_i': _d[2], 'B_w_gate': _d[3], 'B_w_up': _d[4], 'B_w_down': _d[5], **_const})
    _out, _vjp = jax.vjp(_f, A_x, A_w_r, A_w_i, B_w_gate, B_w_up, B_w_down)
    _grads = _vjp(grad_out)
    _out0 = jnp.asarray(_out)
    return (_out0, *[jnp.asarray(_g) for _g in _grads])
```

```python
import numpy as np
import jax
import jax.numpy as jnp
from jax import lax
import jax.experimental.pallas as pl
import jax.experimental.pallas.tpu as pltpu

S, D, F = 2048, 576, 4608
DF = D // 2 + 1
LP = 304
N1, N2 = 16, 128
EPS = 1e-5
BF = 512
BS = 512

f32, bf16 = jnp.float32, jnp.bfloat16


def _dft_constants():
    l = np.arange(DF)[:, None]
    d = np.arange(D)[None, :]
    ang = 2.0 * np.pi * ((l * d) % D) / D
    td = np.zeros((2 * LP, D), np.float64)
    td[:DF] = np.cos(ang)
    td[LP:LP + DF] = -np.sin(ang)
    m = np.zeros((N1, 2 * N2, 2 * N2), np.float64)
    s2 = np.arange(N2)[:, None]
    for k1 in range(N1):
        kk = np.zeros(N2, np.int64)
        for t in range(16):
            for j in range(8):
                kk[(16 * j + k1 + t) % N2] = k1 + N1 * (8 * t + j)
        a = 2.0 * np.pi * ((s2 * kk[None, :]) % S) / S
        mr, mi = np.cos(a), -np.sin(a)
        m[k1] = np.block([[mr, mi], [-mi, mr]])
    cast = lambda v: np.asarray(v, np.float32).astype(bf16)
    return cast(td), cast(td.T.copy()), cast(m)


_TD, _TDT, _M = _dft_constants()

_NT = (((1,), (1,)), ((), ()))


def _dot(a, b):
    return jnp.dot(a, b, preferred_element_type=f32)


def _dot_nt(a, b):
    return lax.dot_general(a, b, _NT, preferred_element_type=f32)


def _cmul_const(z, k, n):
    re, im = z
    k = k % n
    if k == 0:
        return z
    if 4 * k == n:
        return im, -re
    if 2 * k == n:
        return -re, -im
    if 4 * k == 3 * n:
        return -im, re
    c = float(np.cos(2 * np.pi * k / n))
    s = float(-np.sin(2 * np.pi * k / n))
    if abs(c + s) < 1e-12:
        return (re + im) * c, (im - re) * c
    if abs(c - s) < 1e-12:
        return (re - im) * c, (im + re) * c
    return re * c - im * s, re * s + im * c


def _fft(z):
    n = len(z)
    if n == 1:
        return z
    e, o = _fft(z[0::2]), _fft(z[1::2])
    out = [None] * n
    for k in range(n // 2):
        (er, ei), (orr, oi) = e[k], o[k]
        if 4 * k == n:
            out[k] = (er + oi, ei - orr)
            out[k + n // 2] = (er - oi, ei + orr)
        else:
            tr, ti = _cmul_const(o[k], k, n)
            out[k] = (er + tr, ei + ti)
            out[k + n // 2] = (er - tr, ei - ti)
    return out


def _ifft(z):
    o = _fft(z)
    return [o[(-k) % len(z)] for k in range(len(z))]


def _tile(t):
    return slice(t * N2, (t + 1) * N2)


def _skew(tiles):
    lane = lax.broadcasted_iota(jnp.int32, tiles[0].shape, 1)
    cur = [tiles[(-m) % N1] for m in range(N1)]
    for b in range(4):
        mask = (lane & (1 << b)) != 0
        cur = [jnp.where(mask, cur[(m - (1 << b)) % N1], cur[m]) for m in range(N1)]
    return cur


def _ln_stats(v):
    mu = jnp.mean(v, axis=0, keepdims=True)
    c = v - mu
    rstd = lax.rsqrt(jnp.mean(c * c, axis=0, keepdims=True) + EPS)
    return c * rstd, rstd


def _ln_bwd(dn, xhat, rstd):
    m1 = jnp.mean(dn, axis=0, keepdims=True)
    m2 = jnp.mean(dn * xhat, axis=0, keepdims=True)
    return rstd * (dn - m1 - xhat * m2)


def _kernel(xT, wrT, wiT, goT, td, tdT, m, wg, wu, wdT,
            outT, dxT, dwrT, dwiT, dwg, dwu, dwdT,
            hT, hnT, hn, go, oT, dhnT, a_s, dg_s, du_s,
            wr_s, wi_s, x_s, p_s, z_s, b_s):
    j = pl.program_id(0)
    nj = pl.num_programs(0)

    def row_scale(r0, n):
        l = r0 + lax.broadcasted_iota(jnp.int32, (n, N2), 0)
        edge = jnp.logical_or(l == 0, l == DF - 1)
        return jnp.where(edge, 1.0 / (S * D), 2.0 / (S * D)).astype(f32)

    def fwd_front(src):
        for c in range(S // BS):
            cs = slice(c * BS, (c + 1) * BS)
            p_s[:, cs] = _dot(td[...], src[:, cs])

        def body(i, carry):
            r0 = pl.multiple_of(i * 16, 16)
            rr, ri = pl.ds(r0, 16), pl.ds(r0 + LP, 16)
            o = _fft([(p_s[rr, _tile(t)], p_s[ri, _tile(t)]) for t in range(N1)])
            for k in range(N1):
                b_s[k, rr, _tile(0)] = o[k][0].astype(bf16)
                b_s[k, rr, _tile(1)] = o[k][1].astype(bf16)
            return carry
        lax.fori_loop(0, LP // 16, body, 0)

    def inv_stage(k, yr, yi):
        y = jnp.concatenate([yr.astype(bf16), yi.astype(bf16)], axis=1)
        bb = _dot_nt(y, m[k])
        p_s[0:LP, _tile(k)] = bb[:, :N2]
        p_s[LP:2 * LP, _tile(k)] = bb[:, N2:]

    def inv_back():
        def body(i, carry):
            r0 = pl.multiple_of(i * 16, 16)
            rr, ri = pl.ds(r0, 16), pl.ds(r0 + LP, 16)
            o = _ifft([(p_s[rr, _tile(t)], p_s[ri, _tile(t)]) for t in range(N1)])
            for t in range(N1):
                z_s[rr, _tile(t)] = o[t][0].astype(bf16)
                z_s[ri, _tile(t)] = o[t][1].astype(bf16)
            return carry
        lax.fori_loop(0, LP // 16, body, 0)

    @pl.when(j == 0)
    def _():
        for src, dst in ((wrT, wr_s), (wiT, wi_s)):
            dst[DF - 1:LP, :] = jnp.zeros((LP - DF + 1, S), f32)
            dst[0:DF, :] = src[...].astype(f32)

            def wbody(i, carry, dst=dst):
                r0 = pl.multiple_of(i * 8, 8)
                rr = pl.ds(r0, 8)
                sc = row_scale(r0, 8)
                tiles = [dst[rr, _tile(t)] * sc for t in range(N1)]
                tiles = [pltpu.roll(v, t, 1) if t else v for t, v in enumerate(tiles)]
                for k, v in enumerate(_skew(tiles)):
                    dst[rr, _tile(k)] = v
                return carry
            lax.fori_loop(0, LP // 8, wbody, 0)

        for t in range(N1):
            xh, _ = _ln_stats(xT[:, _tile(t)].astype(f32))
            hnT[:, _tile(t)] = xh.astype(bf16)
        fwd_front(hnT)
        for k in range(N1):
            xx = _dot(b_s[k], m[k])
            x_s[k] = xx
            xr, xi = xx[:, :N2], xx[:, N2:]
            wr, wi = wr_s[:, _tile(k)], wi_s[:, _tile(k)]
            inv_stage(k, xr * wr - xi * wi, xr * wi + xi * wr)
        inv_back()
        for c in range(S // BS):
            cs = slice(c * BS, (c + 1) * BS)
            hT[:, cs] = xT[:, cs].astype(f32) + _dot(tdT[...], z_s[:, cs])
        for t in range(N1):
            hh, _ = _ln_stats(hT[:, _tile(t)])
            hnT[:, _tile(t)] = hh.astype(bf16)
        hn[...] = hnT[...].T
        go[...] = goT[...].T
        oT[...] = jnp.zeros_like(oT)
        dhnT[...] = jnp.zeros_like(dhnT)

    def body1(i, carry):
        r = pl.ds(pl.multiple_of(i * BS, BS), BS)
        h = hn[r, :]
        g = _dot(h, wg[...])
        u = _dot(h, wu[...])
        da = _dot(go[r, :], wdT[...])
        sg = jax.nn.sigmoid(g)
        sl = g * sg
        a_s[r, :] = (sl * u).astype(bf16)
        du_s[r, :] = (da * sl).astype(bf16)
        dg_s[r, :] = (da * u * (sg + sl * (1.0 - sg))).astype(bf16)
        return carry
    lax.fori_loop(0, S // BS, body1, 0)

    dwg[...] = _dot(hnT[...], dg_s[...]).astype(bf16)
    dwu[...] = _dot(hnT[...], du_s[...]).astype(bf16)
    dwdT[...] = _dot(goT[...], a_s[...]).astype(bf16)

    def body3(i, carry):
        r = pl.ds(pl.multiple_of(i * BS, BS), BS)
        oT[:, r] += _dot_nt(wdT[...], a_s[r, :])
        dhnT[:, r] += _dot_nt(wg[...], dg_s[r, :]) + _dot_nt(wu[...], du_s[r, :])
        return carry
    lax.fori_loop(0, S // BS, body3, 0)

    @pl.when(j == nj - 1)
    def _():
        for t in range(N1):
            ts = _tile(t)
            h = hT[:, ts]
            outT[:, ts] = (h + oT[:, ts]).astype(bf16)
            hh, rstd = _ln_stats(h)
            dh = goT[:, ts].astype(f32) + _ln_bwd(dhnT[:, ts], hh, rstd)
            hT[:, ts] = dh
            hnT[:, ts] = dh.astype(bf16)
        fwd_front(hnT)
        for k in range(N1):
            gg = _dot(b_s[k], m[k])
            gr, gi = gg[:, :N2], gg[:, N2:]
            wr, wi = wr_s[:, _tile(k)], wi_s[:, _tile(k)]
            xr, xi = x_s[k, :, _tile(0)], x_s[k, :, _tile(1)]
            inv_stage(k, gr * wr + gi * wi, gi * wr - gr * wi)
            wr_s[:, _tile(k)] = gr * xr + gi * xi
            wi_s[:, _tile(k)] = gi * xr - gr * xi
        inv_back()
        for c in range(S // BS):
            cs = slice(c * BS, (c + 1) * BS)
            oT[:, cs] = _dot(tdT[...], z_s[:, cs])
        for t in range(N1):
            ts = _tile(t)
            xh, rstd = _ln_stats(xT[:, ts].astype(f32))
            dxT[:, ts] = (hT[:, ts] + _ln_bwd(oT[:, ts], xh, rstd)).astype(bf16)
        for src, dst in ((wr_s, dwrT), (wi_s, dwiT)):
            def wbody(i, carry, src=src):
                r0 = pl.multiple_of(i * 8, 8)
                rr = pl.ds(r0, 8)
                sc = row_scale(r0, 8)
                tiles = _skew([src[rr, _tile(k)] * sc for k in range(N1)])
                for t, v in enumerate(tiles):
                    src[rr, _tile(t)] = pltpu.roll(v, N2 - t, 1) if t else v
                return carry
            lax.fori_loop(0, LP // 8, wbody, 0)
            dst[...] = src[0:DF, :].astype(bf16)


@jax.jit
def pallas_sequential_preLN__spectral_gfnet__swiglu_ffn__prompt_kernel(
    A_x: jax.Array,
    A_w_r: jax.Array,
    A_w_i: jax.Array,
    B_x: jax.Array,
    B_w_gate: jax.Array,
    B_w_up: jax.Array,
    B_w_down: jax.Array,
    grad_out: jax.Array,
):
    del B_x
    once = lambda shape: pl.BlockSpec(
        shape, lambda j: (0,) * len(shape), pipeline_mode=pl.Buffered(1))
    full = lambda shape: pl.BlockSpec(shape, lambda j: (0,) * len(shape))
    wblk = pl.BlockSpec((D, BF), lambda j: (0, j))
    sds = lambda shape: jax.ShapeDtypeStruct(shape, bf16)
    outs = pl.pallas_call(
        _kernel,
        grid=(F // BF,),
        in_specs=[once((D, S)), once((DF, S)), once((DF, S)), once((D, S)),
                  once(_TD.shape), once(_TDT.shape), once(_M.shape),
                  wblk, wblk, wblk],
        out_specs=[full((D, S)), full((D, S)), full((DF, S)), full((DF, S)),
                   wblk, wblk, wblk],
        out_shape=[sds((D, S)), sds((D, S)), sds((DF, S)), sds((DF, S)),
                   sds((D, F)), sds((D, F)), sds((D, F))],
        scratch_shapes=[
            pltpu.VMEM((D, S), f32),
            pltpu.VMEM((D, S), bf16),
            pltpu.VMEM((S, D), bf16),
            pltpu.VMEM((S, D), bf16),
            pltpu.VMEM((D, S), f32),
            pltpu.VMEM((D, S), f32),
            pltpu.VMEM((S, BF), bf16),
            pltpu.VMEM((S, BF), bf16),
            pltpu.VMEM((S, BF), bf16),
            pltpu.VMEM((LP, S), f32),
            pltpu.VMEM((LP, S), f32),
            pltpu.VMEM((N1, LP, 2 * N2), f32),
            pltpu.VMEM((2 * LP, S), f32),
            pltpu.VMEM((2 * LP, S), bf16),
            pltpu.VMEM((N1, LP, 2 * N2), bf16),
        ],
        compiler_params=pltpu.CompilerParams(
            dimension_semantics=("arbitrary",), vmem_limit_bytes=110 * 2**20),
    )(A_x[0].T, A_w_r.T, A_w_i.T, grad_out[0].T, _TD, _TDT, _M,
      B_w_gate, B_w_up, B_w_down.T)
    outT, dxT, dwrT, dwiT, dwg, dwu, dwdT = outs
    return (outT.T[None], dxT.T[None], dwrT.T, dwiT.T, dwg, dwu, dwdT.T)
```

```python
import numpy as np
import jax
import jax.numpy as jnp
from jax import lax
import jax.experimental.pallas as pl
import jax.experimental.pallas.tpu as pltpu
from functools import partial

S, D, F = 2048, 576, 4608
DF = D // 2 + 1
LP = 304
WN = 352
FR = 0.85
N1, N2 = 16, 128
EPS = 1e-5
BF = 256
BS = 512
NF = F // BF
HS, HD, HF = S // 2, D // 2, BF // 2

f32, bf16 = jnp.float32, jnp.bfloat16

_BASE = (1, 8, 2, 7, 3, 6, 4, 5, 0)


def _dft_constants():
    d2 = np.arange(64)[None, :]

    def cs(base, n):
        a = 2.0 * np.pi * (((base + 9 * np.arange(n))[:, None] * d2) % D) / D
        return np.cos(a), np.sin(a)
    td = np.zeros((5, 128, 128), np.float64)
    for g in range(4):
        c1, s1 = cs(g + 1, 32)
        c2, s2 = cs(8 - g, 32)
        td[g] = np.block([[c1, -s1], [c2, s2], [-s1, -c1], [-s2, c2]])
    c0, s0 = cs(0, 33)
    td[4, 0:33, :64] = c0
    td[4, 48:81, :64] = -s0
    m = np.zeros((N1, 2 * N2, 2 * N2), np.float64)
    s2 = np.arange(N2)[:, None]
    for k1 in range(N1):
        kk = np.zeros(N2, np.int64)
        for t in range(16):
            for j in range(8):
                kk[(16 * j + k1 + t) % N2] = k1 + N1 * (8 * t + j)
        a = 2.0 * np.pi * ((s2 * kk[None, :]) % S) / S
        mr, mi = np.cos(a), -np.sin(a)
        m[k1] = np.block([[mr, mi], [-mi, mr]])
    cast = lambda v: np.asarray(v, np.float32).astype(bf16)
    return cast(td), cast(td.transpose(0, 2, 1).copy()), cast(m)


_TD, _TDT, _M = _dft_constants()
_NT = (((1,), (1,)), ((), ()))


def _dot(a, b):
    return jnp.dot(a, b, preferred_element_type=f32)


def _dot_nt(a, b):
    return lax.dot_general(a, b, _NT, preferred_element_type=f32)


def _cmul_const(z, k, n):
    re, im = z
    if k == 0:
        return z
    c = float(np.cos(2 * np.pi * k / n))
    s = float(-np.sin(2 * np.pi * k / n))
    if abs(c + s) < 1e-12:
        return (re + im) * c, (im - re) * c
    if abs(c - s) < 1e-12:
        return (re - im) * c, (im + re) * c
    return re * c - im * s, re * s + im * c


def _fft(z):
    n = len(z)
    if n == 1:
        return z
    e, o = _fft(z[0::2]), _fft(z[1::2])
    out = [None] * n
    for k in range(n // 2):
        (er, ei), (orr, oi) = e[k], o[k]
        if 4 * k == n:
            out[k] = (er + oi, ei - orr)
            out[k + n // 2] = (er - oi, ei + orr)
        else:
            tr, ti = _cmul_const(o[k], k, n)
            out[k] = (er + tr, ei + ti)
            out[k + n // 2] = (er - tr, ei - ti)
    return out


def _ifft(z):
    o = _fft(z)
    return [o[(-k) % len(z)] for k in range(len(z))]


_C1, _C2, _C4 = (float(np.cos(2 * np.pi * k / 9)) for k in (1, 2, 4))
_S1, _S2, _S3, _S4 = (float(np.sin(2 * np.pi * k / 9)) for k in (1, 2, 3, 4))


def _cosmix(x0, s):
    s1, s2, s3, s4 = s
    u, v, b = x0 + s3, s1 + s2 + s4, x0 - 0.5 * s3
    p, q = s1 - s4, s2 - s4
    m1, m2 = _C1 * p + _C2 * q, _C2 * p + _C4 * q
    return [u + v, b + m1, b + m2, u - 0.5 * v, b - (m1 + m2)]


def _sinmix(t):
    t1, t2, t3, t4 = t
    p, q, h = t1 - t4, t2 + t4, _S3 * t3
    n1, n2 = _S1 * p + _S2 * q, _S2 * p + _S4 * q
    return [n1 + h, n2 - h, _S3 * (t1 - t2 + t4), n2 - n1 + h]


def _dft9(x):
    re = _cosmix(x[0], [x[j] + x[9 - j] for j in range(1, 5)])
    si = _sinmix([x[j] - x[9 - j] for j in range(1, 5)])
    return re, si


def _idft9(re, si):
    p, q = _cosmix(re[0], re[1:]), _sinmix(si)
    lo = [p[j] + q[j - 1] for j in range(1, 5)]
    hi = [p[j] - q[j - 1] for j in range(1, 5)]
    return [p[0]] + lo + hi[::-1]


def _rhs_ops(b11, b12, b21, b22):
    return [b11 + b22, b11, b12 - b22, b21 - b11, b22, b11 + b12, b21 + b22]


def _lhs_ops(a11, a12, a21, a22):
    return [a11 + a22, a21 + a22, a11, a22, a11 + a12, a21 - a11, a12 - a22]


def _combine(m, k):
    if k == 0:
        return m[0] + m[3] - m[4] + m[6]
    if k == 3:
        return m[0] - m[1] + m[2] + m[5]
    return m[2] + m[4] if k == 1 else m[1] + m[3]


def _weave(main, side, fence=None):
    done = 0
    for i, f in enumerate(main):
        res = f()
        if fence is not None:
            fence[12, 0:8, :] = res[-8:, -N2:]
        upto = min(len(side), int((i + 1) * len(side) / (FR * len(main)) + 0.999))
        for g in side[done:upto]:
            g()
        done = upto


def _merge(a, b):
    out = []
    _weave([partial(out.append, f) for f in a], [partial(out.append, f) for f in b])
    return out


def _w_ops(w11, w12, w21, w22):
    return [w11 + w22, w21 - w22, w12 + w22, w11 + w21, w12 - w11, w22, w11]


def _combine_t(n, a):
    if a == 0:
        return n[0] + n[4] - n[5] + n[2], n[1] + n[5]
    return n[6] + n[4], n[0] - n[6] + n[1] + n[3]


def _tile(t):
    return slice(t * N2, (t + 1) * N2)


def _skew(tiles):
    lane = lax.broadcasted_iota(jnp.int32, tiles[0].shape, 1)
    cur = [tiles[(-m) % N1] for m in range(N1)]
    for b in range(4):
        mask = (lane & (1 << b)) != 0
        cur = [jnp.where(mask, cur[(m - (1 << b)) % N1], cur[m]) for m in range(N1)]
    return cur


def _kernel(x_h, wr_h, wi_h, go_h, td_h, tdT_h, m_h, wg_h, wu_h, wd_h,
            out_h, dx_h, dwr_h, dwi_h, dwg_h, dwu_h, dwd_h,
            xT, wrT, wiT, goT, td, tdT, m, w_s, dw_s, ob,
            hT, tmp, hn, go, acc_o, acc_h, q_v, wo_s, ho_s, go_s, ha_s, ga_s, wb_s, pre0, pre1, mp_s,
            st_s, z_s, wr_s, wi_s, x_s, p_s, e_s, b_s, q_s, wn_s, sem, wsem, dsem):
    cp = pltpu.make_async_copy
    c_td, c_wr, c_wi, c_m, c_tdT, c_go = [
        cp(a, b, sem.at[i]) for i, (a, b) in enumerate(
            ((td_h, td), (wr_h, wrT), (wi_h, wiT), (m_h, m), (tdT_h, tdT), (go_h, goT)))]
    c_x = [cp(x_h.at[:, c * 512:(c + 1) * 512], xT.at[:, c * 512:(c + 1) * 512], sem.at[6 + c]) for c in range(4)]

    def fcols(j):
        return pl.ds(j * BF if isinstance(j, int) else pl.multiple_of(j * BF, BF), BF)

    def w_in(j):
        return [cp(src.at[:, fcols(j)], w_s.at[j % 3, i], wsem.at[j % 3, i]) for i, src in enumerate((wg_h, wu_h, wd_h))]

    def dw_out(j):
        return [cp(dw_s.at[j % 2, i], dst.at[:, fcols(j)], dsem.at[j % 2, i]) for i, dst in enumerate((dwg_h, dwu_h, dwd_h))]

    def start(cs):
        for c in cs:
            c.start()

    def wait(cs):
        for c in cs:
            c.wait()

    start(c_x + [c_td])
    z_s[0] = 0
    lo, hi = slice(0, HF), slice(HF, BF)

    def edge_scale(i):
        if i not in (32, 36):
            return 2.0 / (S * D)
        r = lax.broadcasted_iota(jnp.int32, (8, N2), 0)
        return jnp.where(r == 0, 1.0 / (S * D), 2.0 / (S * D)).astype(f32)

    def nat_rows(i):
        return pl.ds(_BASE[min(i // 4, 8)] + 72 * (i - 4 * min(i // 4, 8)), 8, stride=9)

    def colmean(f):
        parts = [f(r) for r in range(0, D, 16)]
        return [jnp.broadcast_to(jnp.sum(sum(p[1:], p[0]), axis=0, keepdims=True) * (1.0 / D), (16, N2))
                for p in zip(*parts)]

    def stats(load, row, t):
        mu, = colmean(lambda r: (load(r),))
        var, = colmean(lambda r: (jnp.square(load(r) - mu),))
        rstd = lax.rsqrt(var + EPS)
        st_s[row, :, _tile(t)] = mu
        st_s[row + 1, :, _tile(t)] = rstd
        return mu, rstd

    def radix9(t, load):
        for c in range(4):
            re, si = _dft9([load(64 * d1 + 16 * c) for d1 in range(9)])
            for g in range(4):
                e_s[g, 16 * c:16 * c + 16, _tile(t)] = re[g + 1].astype(bf16)
                e_s[g, 64 + 16 * c:80 + 16 * c, _tile(t)] = si[g].astype(bf16)
            e_s[4, 16 * c:16 * c + 16, _tile(t)] = re[0].astype(bf16)

    def iradix9(t, store):
        for c in range(4):
            rr, ri = slice(16 * c, 16 * c + 16), slice(64 + 16 * c, 80 + 16 * c)
            y = _idft9([p_s[4, rr, _tile(t)]] + [p_s[g, rr, _tile(t)] for g in range(4)],
                       [p_s[g, ri, _tile(t)] for g in range(4)])
            for d1 in range(9):
                store(64 * d1 + 16 * c, y[d1])

    def slabs():
        for g in range(5):
            n = 64 if g < 4 else 48
            for c in range(0, n, 16):
                yield g, n, c, slice(c, c + 16), slice(n + c, n + c + 16), slice(64 * g + c, 64 * g + c + 16)

    def t_front():
        def run(g, n, c, rr, ri, ro):
            if c == 0:
                kk = 128 if g < 4 else 64
                p_s[g, 0:2 * n, :] = _dot(td[g, 0:2 * n, 0:kk], e_s[g, 0:kk, :])
            o = _fft([(p_s[g, rr, _tile(t)], p_s[g, ri, _tile(t)]) for t in range(N1)])
            for k in range(N1):
                b_s[k, ro, _tile(0)] = o[k][0].astype(bf16)
                b_s[k, ro, _tile(1)] = o[k][1].astype(bf16)
        return [partial(run, *a) for a in slabs()]

    def t_back():
        def run(g, n, c, rr, ri, ro):
            o = _ifft([(q_s[k, ro, _tile(0)], q_s[k, ro, _tile(1)]) for k in range(N1)])
            for t in range(N1):
                e_s[g, rr, _tile(t)] = o[t][0].astype(bf16)
                e_s[g, ri, _tile(t)] = o[t][1].astype(bf16)
            if c + 16 == n:
                mm = 128 if g < 4 else 64
                p_s[g, 0:mm, :] = _dot(tdT[g, 0:mm, 0:2 * n], e_s[g, 0:2 * n, :])
        return [partial(run, *a) for a in slabs()]

    def inv_stage(k, yr, yi):
        y = jnp.concatenate([yr.astype(bf16), yi.astype(bf16)], axis=1)
        q_s[k] = _dot_nt(y, m[k])

    def t_wb(ws):
        def run(v, r):
            quads = [ws[v, r0 + r:r0 + r + 32, cs].astype(f32) for r0 in (0, 256) for cs in (lo, hi)]
            for q, val in enumerate(_rhs_ops(*quads)):
                wb_s[q, r:r + 32, _tile(v)] = val.astype(bf16)
        return [partial(run, v, r) for v in range(3) for r in range(0, 256, 32)]

    def t_wo(ws):
        def run(v, r):
            quads = [ws[v, r0 + r:r0 + r + 32, cs].astype(f32) for r0 in (0, HD) for cs in (lo, hi)]
            for q, val in enumerate(_w_ops(*quads)):
                wo_s[q, r:r + 32, _tile(v)] = val.astype(bf16)
        return [partial(run, v, r) for v in range(3) for r in range(0, HD, 32)]

    def t_pre(ws, i, pre):
        r, r2 = slice(i * BS, (i + 1) * BS), slice(HS + i * BS, HS + (i + 1) * BS)
        out = []
        for v in range(3):
            ops, rem = (ha_s, hn) if v < 2 else (ga_s, go)
            mm = []
            def prod(q, v=v, ops=ops, mm=mm):
                mm.append(_dot(ops[q, r, :], wb_s[q, :, _tile(v)]))
                return mm[-1]
            def fin(k, v=v, rem=rem, mm=mm):
                res = _combine(mm, k) + _dot(rem[(r, r2)[k // 2], :], ws[v, 512:D, (lo, hi)[k % 2]])
                pre[4 * v + k] = res
                return res
            out += [partial(prod, q) for q in range(7)] + [partial(fin, k) for k in range(4)]
        return out

    def t_act(i, pre, z):
        def run(c):
            def act(k):
                g, u, da = (pre[z + 4 * v + k, c:c + 16, :] for v in range(3))
                sg = 0.5 * jnp.tanh(0.5 * g) + 0.5
                sl = g * sg
                return da * u * (sg + sl * (1.0 - sg)), da * sl, sl * u
            def put(q, vals):
                for v in range(3):
                    q_v[q, i * BS + c:i * BS + c + 16, _tile(v)] = vals[v].astype(bf16)
            p11 = act(0)
            put(1, p11)
            p22 = act(3)
            put(4, p22)
            put(0, [a + b for a, b in zip(p11, p22)])
            p = act(1)
            put(2, [a - b for a, b in zip(p, p22)])
            put(5, [a + b for a, b in zip(p11, p)])
            p = act(2)
            put(3, [a - b for a, b in zip(p, p11)])
            put(6, [a + b for a, b in zip(p, p22)])
        return [partial(run, c) for c in range(0, BS, 16)]

    def t_acc(i, first=False):
        r = slice(i * BS, (i + 1) * BS)
        def run(acc, q, cs):
            res = _dot_nt(wo_s[q, :, cs], q_v[q, r, cs])
            if not first:
                res = acc[q, :, r] + res
            acc[q, :, r] = res
            return res
        return [partial(run, acc, q, cs) for q in range(7)
                for acc, cs in ((acc_h, slice(0, BF)), (acc_o, slice(BF, 3 * HF)))]

    def t_dw(i, dst=None):
        r = slice(i * BS, (i + 1) * BS)
        out = []
        for v in range(3):
            mm = []
            def prod(q, v=v, mm=mm):
                res = _dot((ho_s if v < 2 else go_s)[q, :, r], q_v[q, r, _tile(v)])
                if i == 0:
                    mp_s[7 * v + q] = res
                    return res
                mm.append(mp_s[7 * v + q] + res)
                if q == 6:
                    for k in range(4):
                        dst[v, (k // 2) * HD:(k // 2 + 1) * HD, (lo, hi)[k % 2]] = _combine(mm, k).astype(bf16)
                return res
            out += [partial(prod, q) for q in range(7)]
        return out

    def t_skew_in():
        def widen(src):
            for t in range(N1):
                wn_s[t, 0:DF, :] = src[:, _tile(t)].astype(f32)
        def run(dst, i):
            sc = edge_scale(i)
            tiles = [wn_s[t, nat_rows(i), :] * sc for t in range(N1)]
            tiles = [pltpu.roll(v, t, 1) if t else v for t, v in enumerate(tiles)]
            for k, v in enumerate(_skew(tiles)):
                dst[i * 8:i * 8 + 8, _tile(k)] = v
        return [f for src, dst in ((wrT, wr_s), (wiT, wi_s))
                for f in [partial(widen, src)] + [partial(run, dst, i) for i in range(LP // 8 - 1)]]

    def t_skew_out():
        def narrow(dst):
            for t in range(N1):
                dst[:, _tile(t)] = wn_s[t, 0:DF, :].astype(bf16)
        def run(h, i):
            sc = edge_scale(i)
            tiles = _skew([x_s[k, i * 8:i * 8 + 8, _tile(h)] * sc for k in range(N1)])
            for t, v in enumerate(tiles):
                wn_s[t, nat_rows(i), :] = pltpu.roll(v, N2 - t, 1) if t else v
        return [f for h, dst in enumerate((wrT, wiT))
                for f in [partial(run, h, i) for i in range(LP // 8 - 1)] + [partial(narrow, dst)]]

    for c in range(4):
        c_x[c].wait()
        if c == 1:
            start([c_m, c_wr, c_wi, c_tdT])
            wn_s[:, DF - 1:, :] = jnp.zeros((N1, WN - DF + 1, N2), f32)
            wr_s[LP - 8:LP, :] = jnp.zeros((8, S), f32)
            wi_s[LP - 8:LP, :] = jnp.zeros((8, S), f32)
        for t in range(4 * c, 4 * c + 4):
            load = lambda r: xT[r:r + 16, _tile(t)].astype(f32)
            mu, rstd = stats(load, 0, t)
            radix9(t, lambda r: (load(r) - mu) * rstd)
    c_td.wait()
    _weave(t_front(), [])

    def t_h(t):
        def run():
            for a in range(2):
                ts = _tile(t + 8 * a)
                def st(r, v):
                    hT[r:r + 16, ts] = v + xT[r:r + 16, ts].astype(f32)
                iradix9(t + 8 * a, st)
                load = lambda r: hT[r:r + 16, ts]
                mu, rstd = stats(load, 2, t + 8 * a)
                for r in range(0, D, 16):
                    tmp[r:r + 16, ts] = (load(r) - mu) * rstd
            lhs_seq(tmp, t, ha_s, hn)
        return run

    def lhs_seq(src, t, ops, rem):
        ts = (_tile(t), _tile(t + 8))
        for r in (0, 128):
            quads = [src[r0 + r:r0 + r + 128, cs].astype(f32) for cs in ts for r0 in (0, 256)]
            for q, val in enumerate(_lhs_ops(*quads)):
                ops[q, ts[0], r:r + 128] = val.astype(bf16).T
        for cs in ts:
            rem[cs, :] = src[512:D, cs].astype(bf16).T

    def lhs_feat(src, ops, t, r):
        quads = [src[r0 + r:r0 + r + 32, cs].astype(f32) for r0 in (0, HD) for cs in (_tile(t), _tile(t + 8))]
        for q, val in enumerate(_lhs_ops(*quads)):
            ops[q, r:r + 32, _tile(t)] = val.astype(bf16)

    t_g = [partial(lhs_seq, goT, t, ga_s, go) for t in range(8)]
    t_feat = lambda src, ops: [partial(lhs_feat, src, ops, t, r) for t in range(8) for r in range(0, HD, 32)]
    def f_spec(k):
        x_s[k] = _dot(b_s[k], m[k])

    def f_filter(k):
        xr, xi = x_s[k, :, _tile(0)], x_s[k, :, _tile(1)]
        wr, wi = wr_s[:, _tile(k)], wi_s[:, _tile(k)]
        inv_stage(k, xr * wr - xi * wi, xr * wi + xi * wr)

    def zero(acc, q):
        acc[q, :, BS:] = jnp.zeros((HD, HS - BS), f32)

    start([c_go] + w_in(0))
    wait([c_m, c_wr, c_wi])
    _weave([partial(f_spec, k) for k in range(N1)], t_skew_in())
    wait([c_tdT, c_go] + w_in(0))
    start(w_in(1) + w_in(2))
    z = z_s[0]
    ws = w_s.at[0]
    _weave([partial(f_filter, k) for k in range(N1)], t_g + t_wb(ws))
    p0, p1 = t_pre(ws, 0, pre0), t_pre(ws, 1, pre1)
    _weave(t_back(), p0[22:])
    _weave(p1[22:], [t_h(t) for t in range(4)])
    _weave(p0[:22], [t_h(t) for t in range(4, 8)])
    fh, fg = t_feat(tmp, ho_s), t_feat(goT, go_s)
    _weave(p1[:22], t_act(0, pre0, z) + t_wo(ws) + fh[:36], pre0)
    wait(w_in(1))
    _weave(t_acc(0, True), fg + fh[36:] + [partial(zero, a, q) for a in (acc_h, acc_o) for q in range(7)])
    _weave(t_dw(0), t_act(1, pre1, z) + t_wb(w_s.at[1]), pre1)

    def fblock(j, carry):
        z = z_s[0]
        ws = w_s.at[j % 3]
        pl.when(j + 1 < NF)(lambda: wait(w_in(j + 1)))
        pl.when(j + 2 < NF)(lambda: start(w_in(j + 2)))
        pl.when(j >= 3)(lambda: wait(dw_out(j - 3)))
        wb = t_wb(w_s.at[(j + 1) % 3])
        _weave(t_acc(1), [])
        _weave(t_pre(ws, 0, pre0), t_wo(ws))
        _weave(_merge(t_pre(ws, 1, pre1), t_dw(1, dw_s.at[(j - 1) % 2])), t_act(0, pre0, z), pre0)
        _weave(_merge(t_acc(0), t_dw(0)), _merge(t_act(1, pre1, z), wb), pre1)
        start(dw_out(j - 1))
        return carry
    lax.fori_loop(1, NF, fblock, 0)

    wait(dw_out(NF - 3))

    def ln_bwd(dn, xh, rstd):
        m1, m2 = colmean(lambda r: (dn(r), dn(r) * xh(r)))
        return lambda r: rstd * (dn(r) - m1 - xh(r) * m2)

    def t_dh(t):
        for r in range(0, HD, 16):
            oo = [acc_o[q, r:r + 16, _tile(t)] for q in range(7)]
            hh = [acc_h[q, r:r + 16, _tile(t)] for q in range(7)]
            for a in range(2):
                ts = _tile(t + 8 * a)
                for r0, o, h in zip((r, HD + r), _combine_t(oo, a), _combine_t(hh, a)):
                    ob[r0:r0 + 16, ts] = (hT[r0:r0 + 16, ts] + o).astype(bf16)
                    hT[r0:r0 + 16, ts] = h
        for a in range(2):
            ts = _tile(t + 8 * a)
            f = ln_bwd(lambda r: hT[r:r + 16, ts], lambda r: tmp[r:r + 16, ts], st_s[3, :, ts])
            def dh(r):
                v = goT[r:r + 16, ts].astype(f32) + f(r)
                tmp[r:r + 16, ts] = v
                return v
            radix9(t + 8 * a, dh)

    def b_spec(k):
        gg = _dot(b_s[k], m[k])
        gr, gi = gg[:, :N2], gg[:, N2:]
        wr, wi = wr_s[:, _tile(k)], wi_s[:, _tile(k)]
        xr, xi = x_s[k, :, _tile(0)], x_s[k, :, _tile(1)]
        b_s[k, :, _tile(0)] = (gr * wr + gi * wi).astype(bf16)
        b_s[k, :, _tile(1)] = (gi * wr - gr * wi).astype(bf16)
        x_s[k, :, _tile(0)] = gr * xr + gi * xi
        x_s[k, :, _tile(1)] = gi * xr - gr * xi

    def b_inv(k):
        q_s[k] = _dot_nt(b_s[k], m[k])

    dw = t_dw(1, dw_s.at[(NF - 1) % 2])
    _weave([partial(t_dh, t) for t in range(4)], t_acc(1))
    _weave([partial(t_dh, t) for t in range(4, 8)], dw[:14])
    c_out = cp(ob, out_h, sem.at[0])
    c_out.start()
    _weave(t_front(), dw[14:18])
    _weave([partial(b_spec, k) for k in range(N1)], [])
    _weave([partial(b_inv, k) for k in range(N1)], t_skew_out())
    _weave(t_back(), dw[18:])
    start(dw_out(NF - 1))
    done = [c_out, cp(wrT, dwr_h, sem.at[1]), cp(wiT, dwi_h, sem.at[2])]
    start(done[1:])
    for c in range(4):
        cs = slice(c * 512, (c + 1) * 512)
        for t in range(4 * c, 4 * c + 4):
            ts = _tile(t)
            def st(r, v):
                hT[r:r + 16, ts] = v
            iradix9(t, st)
            mu, rstd = st_s[0, :, ts], st_s[1, :, ts]
            f = ln_bwd(lambda r: hT[r:r + 16, ts], lambda r: (xT[r:r + 16, ts].astype(f32) - mu) * rstd, rstd)
            for r in range(0, D, 16):
                goT[r:r + 16, ts] = (tmp[r:r + 16, ts] + f(r)).astype(bf16)
        done.append(cp(goT.at[:, cs], dx_h.at[:, cs], sem.at[6 + c]))
        done[-1].start()
    wait(dw_out(NF - 2) + dw_out(NF - 1) + done)


@jax.jit
def pallas_sequential_preLN__spectral_gfnet__swiglu_ffn__prompt_kernel(
    A_x: jax.Array,
    A_w_r: jax.Array,
    A_w_i: jax.Array,
    B_x: jax.Array,
    B_w_gate: jax.Array,
    B_w_up: jax.Array,
    B_w_down: jax.Array,
    grad_out: jax.Array,
):
    del B_x
    hbm = pl.BlockSpec(memory_space=pl.ANY)
    sds = lambda shape: jax.ShapeDtypeStruct(shape, bf16)
    outs = pl.pallas_call(
        _kernel,
        in_specs=[hbm] * 10,
        out_specs=[hbm] * 7,
        out_shape=[sds((D, S)), sds((D, S)), sds((DF, S)), sds((DF, S)),
                   sds((D, F)), sds((D, F)), sds((D, F))],
        scratch_shapes=[
            pltpu.VMEM((D, S), bf16),
            pltpu.VMEM((DF, S), bf16),
            pltpu.VMEM((DF, S), bf16),
            pltpu.VMEM((D, S), bf16),
            pltpu.VMEM(_TD.shape, bf16),
            pltpu.VMEM(_TDT.shape, bf16),
            pltpu.VMEM(_M.shape, bf16),
            pltpu.VMEM((3, 3, D, BF), bf16),
            pltpu.VMEM((2, 3, D, BF), bf16),
            pltpu.VMEM((D, S), bf16),
            pltpu.VMEM((D, S), f32),
            pltpu.VMEM((D, S), f32),
            pltpu.VMEM((S, D - 512), bf16),
            pltpu.VMEM((S, D - 512), bf16),
            pltpu.VMEM((7, HD, HS), f32),
            pltpu.VMEM((7, HD, HS), f32),
            pltpu.VMEM((7, HS, 3 * HF), bf16),
            pltpu.VMEM((7, HD, 3 * HF), bf16),
            pltpu.VMEM((7, HD, HS), bf16),
            pltpu.VMEM((7, HD, HS), bf16),
            pltpu.VMEM((7, HS, 256), bf16),
            pltpu.VMEM((7, HS, 256), bf16),
            pltpu.VMEM((7, 256, 3 * HF), bf16),
            pltpu.VMEM((13, BS, HF), f32),
            pltpu.VMEM((13, BS, HF), f32),
            pltpu.VMEM((21, HD, HF), f32),
            pltpu.VMEM((4, 16, S), f32),
            pltpu.SMEM((1,), jnp.int32),
            pltpu.VMEM((LP, S), f32),
            pltpu.VMEM((LP, S), f32),
            pltpu.VMEM((N1, LP, 2 * N2), f32),
            pltpu.VMEM((5, 128, S), f32),
            pltpu.VMEM((5, 128, S), bf16),
            pltpu.VMEM((N1, LP, 2 * N2), bf16),
            pltpu.VMEM((N1, LP, 2 * N2), f32),
            pltpu.VMEM((N1, WN, N2), f32),
            pltpu.SemaphoreType.DMA((10,)),
            pltpu.SemaphoreType.DMA((3, 3)),
            pltpu.SemaphoreType.DMA((2, 3)),
        ],
        compiler_params=pltpu.CompilerParams(vmem_limit_bytes=127 * 2**20),
    )(A_x[0].T, A_w_r.T, A_w_i.T, grad_out[0].T, _TD, _TDT, _M,
      B_w_gate, B_w_up, B_w_down.T)
    outT, dxT, dwrT, dwiT, dwg, dwu, dwdT = outs
    return (outT.T[None], dxT.T[None], dwrT.T, dwiT.T, dwg, dwu, dwdT.T)
```
